```python
import os as _os
_os.environ.setdefault("JAX_PLATFORMS", "cpu")
import jax
import jax.numpy as jnp

def _softmax(x, axis=-1):
    return jax.nn.softmax(x, axis=axis)
def _gelu(x):
    return jax.nn.gelu(x, approximate=True)
def _silu(x):
    return jax.nn.silu(x)
def _sigmoid(x):
    return jax.nn.sigmoid(x)
def _layernorm(x, axis=-1, eps=1e-5):
    m = jnp.mean(x, axis=axis, keepdims=True)
    v = jnp.var(x, axis=axis, keepdims=True)
    return (x - m) / jnp.sqrt(v + eps)
def _scatter_add(tgt, idx, src, axis=0):
    return tgt.at[idx].add(src)
def _segment_sum(src, seg, n):
    return jax.ops.segment_sum(src, seg, n)
class _Rng:
    def __init__(self, key):
        self._k = key
    def _next(self):
        self._k, sub = jax.random.split(self._k)
        return sub
    def normal(self, shape):
        return jax.random.normal(self._next(), shape, dtype=jnp.bfloat16)
    def randint(self, lo, hi, shape):
        return jax.random.randint(self._next(), shape, lo, hi, dtype=jnp.int32)
    def uniform(self, shape, lo=0.0, hi=1.0):
        return jax.random.uniform(self._next(), shape, jnp.bfloat16, lo, hi)
    def permutation(self, n):
        return jax.random.permutation(self._next(), n)


kernel_name = 'parallel_sum__softmax_full_mha__moe_arch_mod__prompt'

def setup_inputs():
    _rng = _Rng(jax.random.key(int.from_bytes(__import__("os").urandom(4), "little")))
    _w = (lambda a: (lambda t: t.astype(jnp.bfloat16) if jnp.issubdtype(t.dtype, jnp.floating) else t)(jnp.asarray(a)))
    def _A_setup():
        B, S, D = 1, 2048, 512
        return {
            "x": _w((lambda *s: _rng.normal(s) * 0.05)(B, S, D)),
            "wqkv": _w((lambda *s: _rng.normal(s) * 0.1)(D, 3 * D)),
            "wo": _w((lambda *s: _rng.normal(s) * 0.05)(D, D)),
        }
    _A_in = _A_setup()

    def _B_setup():
        B, S, D, F, C = 1, 2048, 512, 1792, 1
        return {
            "x": _w((lambda *s: _rng.normal(s) * 0.05)(B, S, D)),
            "w_r": _w((lambda *s: _rng.normal(s) * 1.6)(D)),
            "w_gate": _w((lambda *s: _rng.normal(s) * 0.1)(D, F)),
            "w_up": _w((lambda *s: _rng.normal(s) * 0.1)(D, F)),
            "w_down": _w((lambda *s: _rng.normal(s) * 0.1)(F, D)),
        }
    _B_in = _B_setup()

    return {
        "A_x": _A_in["x"],
        "A_wqkv": _A_in["wqkv"],
        "A_wo": _A_in["wo"],
        "B_x": _B_in["x"],
        "B_w_r": _B_in["w_r"],
        "B_w_gate": _B_in["w_gate"],
        "B_w_up": _B_in["w_up"],
        "B_w_down": _B_in["w_down"],
    }

def reference(A_x, A_wqkv, A_wo, B_x, B_w_r, B_w_gate, B_w_up, B_w_down):
    def _A_ref(x, wqkv, wo):
        B, S, D = x.shape
        H = 32; Dh = D // H
        qkv = (lambda x, *d: x.transpose(*d))((x @ wqkv).reshape(B, S, 3, H, Dh), 2, 0, 3, 1, 4)
        q, k, v = qkv[0], qkv[1], qkv[2]
        scale = Dh ** -0.5
        scores = jnp.einsum("bhqd,bhkd->bhqk", q, k) * scale
        p = _softmax(scores, axis=-1)
        o = jnp.einsum("bhqk,bhkd->bhqd", p, v)
        return (lambda x, *d: x.transpose(*d))(o, 0, 2, 1, 3).reshape(B, S, D) @ wo

    def _B_ref(x, w_r, w_gate, w_up, w_down):
        B, S, D = x.shape
        C = 1
        r = x @ w_r
        idx = jnp.argsort(-r, axis=-1)[:, :C]
        idx_e = jnp.repeat(idx.reshape(B, C, 1), D, axis=2)
        x_sel = jnp.take_along_axis(x, idx_e, axis=1)
        g = _silu(x_sel @ w_gate)
        u = x_sel @ w_up
        y = (g * u) @ w_down
        r_sel = _sigmoid(jnp.take_along_axis(r, idx, axis=1))
        y = y * r_sel.reshape(B, C, 1)
        b_off = (jnp.arange(B) * S).reshape(B, 1)
        flat_idx = (idx + b_off).reshape(B * C)
        zero = (x * 0.0).reshape(B * S, D)
        upd = _scatter_add(zero, flat_idx, y.reshape(B * C, D), axis=0)
        return x + upd.reshape(B, S, D)

    x = A_x
    xn = _layernorm(x, axis=-1)
    return x + _A_ref(xn, A_wqkv, A_wo) + _B_ref(xn, B_w_r, B_w_gate, B_w_up, B_w_down)
```

```python
import functools, os
import jax
import jax.numpy as jnp
import numpy as np
from jax import lax
import jax.experimental.pallas as pl
import jax.experimental.pallas.tpu as pltpu

S, D, H, DH, F = 2048, 512, 32, 16, 1792
TQ = int(os.environ.get('TQ', 512))
CK = int(os.environ.get('CK', 128))
LAG = int(os.environ.get('LAG', 3))
DEP = int(os.environ.get('DEP', 2))
HN = int(os.environ.get('HN', 2))
NW = int(os.environ.get('NW', 1))
NTI = int(os.environ.get('NTI', 4))
XC = int(os.environ.get('XC', 256))
NX = S // XC
NQ = S // TQ
NC = S // CK
NT_ = H * NQ
LOG2E = 1.4426950408889634
EPS_B = float(np.asarray(jnp.asarray(1e-5, jnp.bfloat16).astype(jnp.float32)))
NT = (((1,), (1,)), ((), ()))


def _kernel(x_hbm, wqkv_hbm, wo_hbm, wr_hbm, wg_hbm, wu_hbm, wd_hbm, o_hbm,
            x_ref, wqkv_ref, wo_ref, wr_ref, wg_ref, wu_ref, wd_ref, out_scr,
            xn_scr, q_scr, k_scr, vT_scr, oT_scr, sA, sB, r_scr, i_scr, sem_x, sem_w, sem_o):
    f32, bf16 = jnp.float32, jnp.bfloat16
    rb = lambda t: t.astype(bf16).astype(f32)

    x_cp = [pltpu.make_async_copy(x_hbm.at[pl.ds(c * XC, XC)], x_ref.at[pl.ds(c * XC, XC)], sem_x.at[c])
            for c in range(NX)]
    w_cp = [pltpu.make_async_copy(src, dst, sem_w.at[i]) for i, (src, dst) in enumerate(
        [(wqkv_hbm, wqkv_ref), (wr_hbm, wr_ref), (wo_hbm, wo_ref), (wg_hbm, wg_ref), (wu_hbm, wu_ref), (wd_hbm, wd_ref)])]
    x_cp[0].start()
    w_cp[0].start()
    w_cp[1].start()
    for c in range(1, NX):
        x_cp[c].start()

    def ln_chunk(c):
        rows = pl.ds(c * XC, XC)
        xf = x_ref[rows, :].astype(f32)
        mean = jnp.sum(xf, axis=-1, keepdims=True) * (1.0 / D)
        cc = xf - mean
        var = jnp.sum(cc * cc, axis=-1, keepdims=True) * (1.0 / D)
        den = rb(jnp.sqrt(rb(rb(var) + EPS_B)))
        xn = rb(rb(xf - rb(mean)) / den)
        xn_scr[rows, :] = xn.astype(bf16)
        rc = rb(jnp.sum(xn * wr_ref[...].astype(f32), axis=-1, keepdims=True))
        rowc = lax.broadcasted_iota(jnp.int32, (XC, 1), 0) + c * XC
        if c == 0:
            r_scr[...] = rc
            i_scr[...] = rowc
        else:
            rrun = r_scr[...]
            better = rc > rrun
            r_scr[...] = jnp.where(better, rc, rrun)
            i_scr[...] = jnp.where(better, rowc, i_scr[...])

    def qkv_chunk(c):
        rows = pl.ds(c * XC, XC)
        xnb = xn_scr[rows, :]
        q = jnp.dot(xnb, wqkv_ref[:, 0:D], preferred_element_type=f32)
        q_scr[:, rows] = (q * (0.25 * LOG2E)).T.astype(bf16)
        k = jnp.dot(xnb, wqkv_ref[:, D:2 * D], preferred_element_type=f32).astype(bf16)
        for h in range(H):
            k_scr[h, pl.ds(c * (XC // 2), XC // 2), :] = pltpu.bitcast(k[:, h * DH:(h + 1) * DH], jnp.int32)
        v = jnp.dot(xnb, wqkv_ref[:, 2 * D:3 * D], preferred_element_type=f32)
        vT_scr[:, rows] = v.T.astype(bf16)

    x_cp[0].wait()
    w_cp[1].wait()
    ln_chunk(0)
    w_cp[0].wait()
    for c in range(NX - 1):
        if c < NW:
            x_cp[c + 1].wait()
        elif c == NW:
            for c2 in range(c + 1, NX):
                x_cp[c2].wait()
        if c == min(NW, NX - 2):
            for cp in w_cp[2:]:
                cp.start()
        ln_chunk(c + 1)
        qkv_chunk(c)
    for cp in w_cp[2:]:
        cp.wait()

    r = r_scr[...]
    rmax = jnp.max(r, axis=0, keepdims=True)
    idx = jnp.min(jnp.where(r == rmax, i_scr[...], S))
    base = pl.multiple_of((idx // 16) * 16, 16)
    blk = xn_scr[pl.ds(base, 16), :]
    sel16 = lax.broadcasted_iota(jnp.int32, (16, 1), 0) == (idx - base)
    xs = jnp.where(sel16, blk, jnp.zeros_like(blk))

    qkv_chunk(NX - 1)

    def qk_setup(t):
        t = jnp.minimum(t, NT_ - 1)
        h = t // NQ
        qi = t % NQ
        qoff = pl.multiple_of(qi * TQ, TQ)
        qt = q_scr[pl.ds(pl.multiple_of(h * DH, DH), DH), pl.ds(qoff, TQ)]
        return h, qt

    def qk_chunk(setup, buf, ci, mpart):
        h, qt = setup
        cs = ci * CK
        kh = pltpu.bitcast(k_scr[h, cs // 2:(cs + CK) // 2, :], bf16)
        s = jnp.dot(kh, qt, preferred_element_type=f32)
        buf[cs:cs + CK, :] = s
        for j in range(CK // 8):
            sj = s[j * 8:(j + 1) * 8, :]
            mpart = sj if mpart is None else jnp.maximum(mpart, sj)
        return mpart

    FP = 256
    NFP = F // FP
    hparts = []
    ypart = None
    st0 = qk_setup(0)
    st1 = qk_setup(1)
    m0 = None
    m1 = None
    for ci in range(NC + LAG):
        if ci < NC:
            m0 = qk_chunk(st0, sA, ci, m0)
        else:
            m1 = qk_chunk(st1, sB, ci - NC, m1)
        if ci < NFP:
            cols = slice(ci * FP, (ci + 1) * FP)
            gg = rb(jnp.dot(xs, wg_ref[:, cols], preferred_element_type=f32))
            gg = rb(gg * jax.nn.sigmoid(gg))
            uu = rb(jnp.dot(xs, wu_ref[:, cols], preferred_element_type=f32))
            hparts.append((gg * uu).astype(bf16))
        elif ci < 2 * NFP:
            j = ci - NFP
            yj = jnp.dot(hparts[j], wd_ref[j * FP:(j + 1) * FP, :], preferred_element_type=f32)
            ypart = yj if ypart is None else ypart + yj
    y = rb(jnp.sum(ypart, axis=0, keepdims=True)) * rb(jax.nn.sigmoid(rmax))

    def fin_max(mpart):
        return jnp.broadcast_to(jnp.max(mpart, axis=0, keepdims=True), (8, TQ))

    def body(i, carry):
        m8n, mO = carry
        t = NTI * i
        setups = [qk_setup(t + 1 + j) for j in range(NTI + 1)]
        bufs = [sB if j % 2 == 0 else sA for j in range(NTI + 1)]
        mp = [mO] + [None] * NTI
        hist = []
        lpart = None
        for pos in range(NTI * NC):
            g = pos + LAG
            ti, ci = g // NC, g % NC
            mp[ti] = qk_chunk(setups[ti], bufs[ti], ci, mp[ti])
            hist.append(mp[ti])
            si, ci = pos // NC, pos % NC
            if ci == 0:
                ts = t + si
                h2 = ts // NQ
                q2off = pl.multiple_of((ts % NQ) * TQ, TQ)
                hoff = pl.multiple_of(h2 * DH, DH)
                m8 = m8n
                lprev = lpart
                lpart = None
                acc = None
                cur = sA if si % 2 == 0 else sB
            cs = ci * CK
            w = None
            if pos - DEP >= 0:
                hd = hist[pos - DEP]
                if ci - DEP == NC - 1 - LAG:
                    m8n = fin_max(hd)
                    hd = m8n
                w = pltpu.bitcast(hd, jnp.int32)
            lp = lpart if lpart is not None else lprev
            if lp is not None:
                lb = pltpu.bitcast(lp, jnp.int32)
                w = lb if w is None else w | lb
            mc8 = m8
            if w is not None:
                z = lax.shift_right_logical(w, 31) & 2
                mc8 = pltpu.bitcast(pltpu.bitcast(m8, jnp.int32) ^ z, f32)
            sc = cur[cs:cs + CK, :].reshape(CK // 8, 8, TQ)
            if ci == 1:
                z2 = lax.shift_right_logical(pltpu.bitcast(acc[0:8], jnp.int32), 31) & 2
                mc8b = pltpu.bitcast(pltpu.bitcast(mc8, jnp.int32) ^ z2, f32)
                hn = HN
                p3 = jnp.concatenate([jnp.exp2(sc[:hn] - mc8b[None]), jnp.exp2(sc[hn:] - mc8[None])], axis=0) if hn < CK // 8 else jnp.exp2(sc - mc8b[None])
            else:
                p3 = jnp.exp2(sc - mc8[None])
            for j in reversed(range(CK // 8)):
                lpart = p3[j] if lpart is None else lpart + p3[j]
            p = p3.reshape(CK, TQ)
            vt = vT_scr[pl.ds(hoff, DH), cs:cs + CK]
            o = jnp.dot(vt, p.astype(bf16), preferred_element_type=f32)
            acc = o if acc is None else acc + o
            if ci == NC - 1:
                l = jnp.sum(lpart, axis=0, keepdims=True)
                oT_scr[pl.ds(hoff, DH), pl.ds(q2off, TQ)] = acc / l
        return m8n, mp[NTI]

    lax.fori_loop(0, NT_ // NTI, body, (fin_max(m0), m1))

    o_cp = [pltpu.make_async_copy(out_scr.at[pl.ds(c * XC, XC)], o_hbm.at[pl.ds(c * XC, XC)], sem_o.at[c])
            for c in range(NX)]
    for c in range(NX):
        rows = pl.ds(c * XC, XC)
        o = oT_scr[:, rows].T.astype(bf16)
        a = jnp.dot(o, wo_ref[...], preferred_element_type=f32)
        rowc = lax.broadcasted_iota(jnp.int32, (XC, 1), 0) + c * XC
        upd = jnp.where(rowc == idx, y, 0.0)
        out_scr[rows, :] = (x_ref[rows, :].astype(f32) + a + (xn_scr[rows, :].astype(f32) + upd)).astype(bf16)
        o_cp[c].start()
    for c in range(NX):
        o_cp[c].wait()


@jax.jit
def pallas_parallel_sum__softmax_full_mha__moe_arch_mod__prompt_kernel(
    A_x, A_wqkv, A_wo, B_x, B_w_r, B_w_gate, B_w_up, B_w_down):
    x = A_x.reshape(S, D)
    wr = B_w_r.reshape(1, D)
    bf16 = jnp.bfloat16
    out = pl.pallas_call(
        _kernel,
        out_shape=jax.ShapeDtypeStruct((S, D), bf16),
        in_specs=[pl.BlockSpec(memory_space=pl.ANY)] * 7,
        out_specs=pl.BlockSpec(memory_space=pl.ANY),
        scratch_shapes=[
            pltpu.VMEM((S, D), bf16),
            pltpu.VMEM((D, 3 * D), bf16),
            pltpu.VMEM((D, D), bf16),
            pltpu.VMEM((1, D), bf16),
            pltpu.VMEM((D, F), bf16),
            pltpu.VMEM((D, F), bf16),
            pltpu.VMEM((F, D), bf16),
            pltpu.VMEM((S, D), bf16),
            pltpu.VMEM((S, D), bf16),
            pltpu.VMEM((D, S), bf16),
            pltpu.VMEM((H, S // 2, DH), jnp.int32),
            pltpu.VMEM((D, S), bf16),
            pltpu.VMEM((D, S), jnp.float32),
            pltpu.VMEM((S, TQ), jnp.float32),
            pltpu.VMEM((S, TQ), jnp.float32),
            pltpu.VMEM((XC, 1), jnp.float32),
            pltpu.VMEM((XC, 1), jnp.int32),
            pltpu.SemaphoreType.DMA((NX,)),
            pltpu.SemaphoreType.DMA((6,)),
            pltpu.SemaphoreType.DMA((NX,)),
        ],
        compiler_params=pltpu.CompilerParams(vmem_limit_bytes=100 * 1024 * 1024),
    )(x, A_wqkv, A_wo, wr, B_w_gate, B_w_up, B_w_down)
    return out.reshape(1, S, D)
```

```python
import jax
import jax.numpy as jnp
from jax import lax
import jax.experimental.pallas as pl
import jax.experimental.pallas.tpu as pltpu

S, D, H, DH, F = 2048, 512, 32, 16, 1792
TQ = 512
CK = 128
LAG = 3
DEP = 2
HN = 2
NTI = 6
NL = 2
XC = 256
FP = 256
NX = S // XC
NQ = S // TQ
NC = S // CK
NFP = F // FP
NT_ = H * NQ
OUT_CHUNKS = [(c * XC, XC) for c in range(NX - 1)] + [(S - XC, XC // 2), (S - XC // 2, XC // 2)]
LOG2E = 1.4426950408889634
EPS_B = 1.0013580322265625e-05
assert (NT_ - NL) % NTI == 0 and NTI % 2 == 0


def _kernel(x_hbm, wqkv_hbm, wo_hbm, wr_hbm, wg_hbm, wu_hbm, wd_hbm, o_hbm,
            x_ref, wqkv_ref, wo_ref, wr_ref, wg_ref, wu_ref, wd_ref, out_scr,
            xn_scr, q_scr, k_scr, vT_scr, oT_scr, sA, sB, r_scr, i_scr, sem_x, sem_w, sem_o):
    f32, bf16, i32 = jnp.float32, jnp.bfloat16, jnp.int32
    rb = lambda t: t.astype(bf16).astype(f32)

    def zero_dep(bits):
        return lax.shift_right_logical(bits, 31) & 2

    x_cp = [pltpu.make_async_copy(x_hbm.at[pl.ds(c * XC, XC)], x_ref.at[pl.ds(c * XC, XC)], sem_x.at[c])
            for c in range(NX)]
    wqkv_cp = [pltpu.make_async_copy(wqkv_hbm.at[:, pl.ds(j * D, D)], wqkv_ref.at[:, pl.ds(j * D, D)], sem_w.at[j])
               for j in range(3)]
    wr_cp = pltpu.make_async_copy(wr_hbm, wr_ref, sem_w.at[3])
    w_cp = [pltpu.make_async_copy(src, dst, sem_w.at[4 + i]) for i, (src, dst) in enumerate(
        [(wo_hbm, wo_ref), (wg_hbm, wg_ref), (wu_hbm, wu_ref), (wd_hbm, wd_ref)])]
    o_cp = [pltpu.make_async_copy(out_scr.at[pl.ds(r0, n)], o_hbm.at[pl.ds(r0, n)], sem_o.at[c])
            for c, (r0, n) in enumerate(OUT_CHUNKS)]

    def ln_chunk(c, dep=None):
        rows = pl.ds(c * XC, XC)
        xf = x_ref[rows, :].astype(f32)
        if dep is not None:
            z = jnp.concatenate([zero_dep(pltpu.bitcast(dep, i32))] * (D // 128), axis=1)
            xf = pltpu.bitcast(pltpu.bitcast(xf, i32).reshape(XC // 8, 8, D) ^ z[None], f32).reshape(XC, D)
        mean = jnp.sum(xf, axis=-1, keepdims=True) * (1.0 / D)
        cc = xf - mean
        var = jnp.sum(cc * cc, axis=-1, keepdims=True) * (1.0 / D)
        den = rb(jnp.sqrt(rb(rb(var) + EPS_B)))
        xn = rb(rb(xf - rb(mean)) / den)
        xn_scr[rows, :] = xn.astype(bf16)
        rc = rb(jnp.sum(xn * wr_ref[...].astype(f32).reshape(1, D), axis=-1, keepdims=True))
        rowc = lax.broadcasted_iota(i32, (XC, 1), 0) + c * XC
        if c == 0:
            r_scr[...] = rc
            i_scr[...] = rowc
        else:
            rrun = r_scr[...]
            better = rc > rrun
            r_scr[...] = jnp.where(better, rc, rrun)
            i_scr[...] = jnp.where(better, rowc, i_scr[...])

    def q_chunk(c):
        rows = pl.ds(c * XC, XC)
        q = jnp.dot(xn_scr[rows, :], wqkv_ref[:, 0:D], preferred_element_type=f32)
        q_scr[:, rows] = (q * (DH ** -0.5 * LOG2E)).T.astype(bf16)

    def kv_chunk(c):
        rows = pl.ds(c * XC, XC)
        xnb = xn_scr[rows, :]
        k = jnp.dot(xnb, wqkv_ref[:, D:2 * D], preferred_element_type=f32).astype(bf16)
        for h in range(H):
            k_scr[h, pl.ds(c * (XC // 2), XC // 2), :] = pltpu.bitcast(k[:, h * DH:(h + 1) * DH], i32)
        v = jnp.dot(xnb, wqkv_ref[:, 2 * D:3 * D], preferred_element_type=f32)
        vT_scr[:, rows] = v.T.astype(bf16)
        return v[0:8, 0:128]

    x_cp[0].start()
    wr_cp.start()
    wqkv_cp[0].start()
    x_cp[0].wait()
    wr_cp.wait()
    x_cp[1].start()
    wqkv_cp[1].start()
    wqkv_cp[2].start()
    ln_chunk(0)
    wqkv_cp[0].wait()
    x_cp[1].wait()
    ln_chunk(1)
    q_chunk(0)
    wqkv_cp[1].wait()
    wqkv_cp[2].wait()
    for c in range(2, NX):
        x_cp[c].start()
    kv_chunk(0)
    q_chunk(1)
    for c in range(2, NX):
        x_cp[c].wait()
    for cp in w_cp:
        cp.start()
    ln_chunk(2)
    vdep = kv_chunk(1)
    for c in range(2, NX):
        if c + 1 < NX:
            ln_chunk(c + 1, vdep)
        q_chunk(c)
        vdep = kv_chunk(c)

    r = r_scr[...]
    rmax = jnp.max(r, axis=0, keepdims=True)
    idx = jnp.minimum(jnp.min(jnp.where(r == rmax, i_scr[...], S)), S - 1)
    base = pl.multiple_of((idx // 16) * 16, 16)
    blk = xn_scr[pl.ds(base, 16), :]
    sel16 = lax.broadcasted_iota(i32, (16, 1), 0) == (idx - base)
    xs = jnp.where(sel16, blk, jnp.zeros_like(blk))
    moe = {'h': [], 'y': None}

    def moe_step(k):
        if k < NFP:
            cols = slice(k * FP, (k + 1) * FP)
            gg = rb(jnp.dot(xs, wg_ref[:, cols], preferred_element_type=f32))
            gg = rb(gg * jax.nn.sigmoid(gg))
            uu = rb(jnp.dot(xs, wu_ref[:, cols], preferred_element_type=f32))
            moe['h'].append((gg * uu).astype(bf16))
        else:
            j = k - NFP
            yj = jnp.dot(moe['h'][j], wd_ref[j * FP:(j + 1) * FP, :], preferred_element_type=f32)
            moe['y'] = yj if moe['y'] is None else moe['y'] + yj
            if k == 2 * NFP - 1:
                moe['y'] = rb(rb(jnp.sum(moe['y'], axis=0, keepdims=True)) * rb(jax.nn.sigmoid(rmax)))

    def out_chunk(c):
        r0, n = OUT_CHUNKS[c]
        rows = pl.ds(r0, n)
        o = oT_scr[:, rows].T.astype(bf16)
        a = jnp.dot(o, wo_ref[...], preferred_element_type=f32)
        rowc = lax.broadcasted_iota(i32, (n, 1), 0) + r0
        upd = jnp.where(rowc == idx, moe['y'], 0.0)
        out_scr[rows, :] = (x_ref[rows, :].astype(f32) + a + (xn_scr[rows, :].astype(f32) + upd)).astype(bf16)
        o_cp[c].start()

    def qk_setup(t):
        h = t // NQ
        qi = t % NQ
        if isinstance(t, int):
            return h, q_scr[h * DH:(h + 1) * DH, qi * TQ:(qi + 1) * TQ]
        qoff = pl.multiple_of(qi * TQ, TQ)
        return h, q_scr[pl.ds(pl.multiple_of(h * DH, DH), DH), pl.ds(qoff, TQ)]

    def qk_chunk(setup, buf, ci, mpart):
        h, qt = setup
        cs = ci * CK
        kh = pltpu.bitcast(k_scr[h, cs // 2:(cs + CK) // 2, :], bf16)
        s = jnp.dot(kh, qt, preferred_element_type=f32)
        buf[cs:cs + CK, :] = s
        for j in range(CK // 8):
            sj = s[j * 8:(j + 1) * 8, :]
            mpart = sj if mpart is None else jnp.maximum(mpart, sj)
        return mpart

    def fin_max(mpart):
        return jnp.broadcast_to(jnp.max(mpart, axis=0, keepdims=True), (8, TQ))

    st0 = qk_setup(0)
    st1 = qk_setup(1)
    m0 = None
    m1 = None
    for ci in range(NC + LAG):
        if ci < NC:
            m0 = qk_chunk(st0, sA, ci, m0)
        else:
            m1 = qk_chunk(st1, sB, ci - NC, m1)

    def run(t, carry, last):
        m8n, mO = carry
        nt = NL if last else NTI
        nqk = nt - 1 if last else nt + 1
        setups = [qk_setup(t + 1 + j) for j in range(nqk)]
        bufs = [sB if j % 2 == 0 else sA for j in range(nqk)]
        mp = [mO] + [None] * nt
        hist = []
        lpart = None
        ndone = 0
        for pos in range(nt * NC):
            g = pos + LAG
            ti, ci = g // NC, g % NC
            if last and pos < 2 * NFP:
                moe_step(pos)
            if ti < nqk:
                mp[ti] = qk_chunk(setups[ti], bufs[ti], ci, mp[ti])
                hist.append(mp[ti])
            else:
                hist.append(None)
                k = g - nqk * NC
                avail = ((pos // NC) + (NQ - nt)) * (TQ // XC)
                if k % 3 == 0 and ndone < avail and pos >= 2 * NFP:
                    out_chunk(ndone)
                    ndone += 1
            si, ci = pos // NC, pos % NC
            if ci == 0:
                ts = t + si
                h2 = ts // NQ
                if last:
                    hsl = slice(h2 * DH, (h2 + 1) * DH)
                    qsl = slice((ts % NQ) * TQ, (ts % NQ + 1) * TQ)
                else:
                    hsl = pl.ds(pl.multiple_of(h2 * DH, DH), DH)
                    qsl = pl.ds(pl.multiple_of((ts % NQ) * TQ, TQ), TQ)
                m8 = m8n
                lprev = lpart
                lpart = None
                acc = None
                cur = sA if si % 2 == 0 else sB
            cs = ci * CK
            w = None
            if pos - DEP >= 0 and hist[pos - DEP] is not None:
                hd = hist[pos - DEP]
                if ci - DEP == NC - 1 - LAG:
                    m8n = fin_max(hd)
                    hd = m8n
                w = pltpu.bitcast(hd, i32)
            lp = lpart if lpart is not None else lprev
            if lp is not None:
                lb = pltpu.bitcast(lp, i32)
                w = lb if w is None else w | lb
            if last and pos == 2 * NFP + 1:
                w = w | pltpu.bitcast(jnp.broadcast_to(moe['y'], (8, TQ)), i32)
            mc8 = m8
            if w is not None:
                mc8 = pltpu.bitcast(pltpu.bitcast(m8, i32) ^ zero_dep(w), f32)
            sc = cur[cs:cs + CK, :].reshape(CK // 8, 8, TQ)
            if ci == 1:
                mc8b = pltpu.bitcast(pltpu.bitcast(mc8, i32) ^ zero_dep(pltpu.bitcast(acc[0:8], i32)), f32)
                p3 = jnp.concatenate([jnp.exp2(sc[:HN] - mc8b[None]), jnp.exp2(sc[HN:] - mc8[None])], axis=0)
            else:
                p3 = jnp.exp2(sc - mc8[None])
            for j in reversed(range(CK // 8)):
                lpart = p3[j] if lpart is None else lpart + p3[j]
            p = p3.reshape(CK, TQ)
            o = jnp.dot(vT_scr[hsl, cs:cs + CK], p.astype(bf16), preferred_element_type=f32)
            acc = o if acc is None else acc + o
            if ci == NC - 1:
                l = jnp.sum(lpart, axis=0, keepdims=True)
                oT_scr[hsl, qsl] = acc / l
        if last:
            return ndone
        return m8n, mp[nt]

    carry = lax.fori_loop(0, (NT_ - NL) // NTI, lambda i, c: run(NTI * i, c, False), (fin_max(m0), m1))
    for cp in w_cp:
        cp.wait()
    ndone = run(NT_ - NL, carry, True)
    for c in range(ndone, len(OUT_CHUNKS)):
        out_chunk(c)
    for cp in o_cp:
        cp.wait()


@jax.jit
def pallas_parallel_sum__softmax_full_mha__moe_arch_mod__prompt_kernel(
    A_x: jax.Array,
    A_wqkv: jax.Array,
    A_wo: jax.Array,
    B_x: jax.Array,
    B_w_r: jax.Array,
    B_w_gate: jax.Array,
    B_w_up: jax.Array,
    B_w_down: jax.Array,
):
    del B_x
    bf16 = jnp.bfloat16
    out = pl.pallas_call(
        _kernel,
        out_shape=jax.ShapeDtypeStruct((S, D), bf16),
        in_specs=[pl.BlockSpec(memory_space=pl.ANY)] * 7,
        out_specs=pl.BlockSpec(memory_space=pl.ANY),
        scratch_shapes=[
            pltpu.VMEM((S, D), bf16),
            pltpu.VMEM((D, 3 * D), bf16),
            pltpu.VMEM((D, D), bf16),
            pltpu.VMEM((D,), bf16),
            pltpu.VMEM((D, F), bf16),
            pltpu.VMEM((D, F), bf16),
            pltpu.VMEM((F, D), bf16),
            pltpu.VMEM((S, D), bf16),
            pltpu.VMEM((S, D), bf16),
            pltpu.VMEM((D, S), bf16),
            pltpu.VMEM((H, S // 2, DH), jnp.int32),
            pltpu.VMEM((D, S), bf16),
            pltpu.VMEM((D, S), jnp.float32),
            pltpu.VMEM((S, TQ), jnp.float32),
            pltpu.VMEM((S, TQ), jnp.float32),
            pltpu.VMEM((XC, 1), jnp.float32),
            pltpu.VMEM((XC, 1), jnp.int32),
            pltpu.SemaphoreType.DMA((NX,)),
            pltpu.SemaphoreType.DMA((8,)),
            pltpu.SemaphoreType.DMA((len(OUT_CHUNKS),)),
        ],
        compiler_params=pltpu.CompilerParams(vmem_limit_bytes=100 * 1024 * 1024),
    )(A_x.reshape(S, D), A_wqkv, A_wo, B_w_r, B_w_gate, B_w_up, B_w_down)
    return out.reshape(1, S, D)
```

```python
import jax
import jax.numpy as jnp
from jax import lax
import jax.experimental.pallas as pl
import jax.experimental.pallas.tpu as pltpu

S, D, H, DH, F = 2048, 512, 32, 16, 1792
TQ = 512
CK = 128
LAG = 3
DEP = 2
HN = 2
NTI = 6
NL = 2
XC = 256
FP = 256
NX = S // XC
NQ = S // TQ
NC = S // CK
NFP = F // FP
NT_ = H * NQ
OUT_CHUNKS = [(c * XC, XC) for c in range(NX - 1)] + [(S - XC, XC // 2), (S - XC // 2, XC // 2)]
EPS_B = 1.0013580322265625e-05
assert (NT_ - NL) % NTI == 0 and NTI % 2 == 0


def _kernel(x_hbm, wqkv_hbm, wo_hbm, wr_hbm, wg_hbm, wu_hbm, wd_hbm, o_hbm,
            x_ref, wqkv_ref, wo_ref, wr_ref, wg_ref, wu_ref, wd_ref, out_scr,
            xn_scr, q_scr, k_scr, vT_scr, oT_scr, sA, sB, r_scr, i_scr, sem_x, sem_w, sem_o):
    f32, bf16, i32 = jnp.float32, jnp.bfloat16, jnp.int32
    rb = lambda t: t.astype(bf16).astype(f32)

    def zero_dep(bits):
        return lax.shift_right_logical(bits, 31) & 2

    x_cp = [pltpu.make_async_copy(x_hbm.at[pl.ds(c * XC, XC)], x_ref.at[pl.ds(c * XC, XC)], sem_x.at[c])
            for c in range(NX)]
    wqkv_cp = [pltpu.make_async_copy(wqkv_hbm.at[:, pl.ds(j * D, D)], wqkv_ref.at[:, pl.ds(j * D, D)], sem_w.at[j])
               for j in range(3)]
    wr_cp = pltpu.make_async_copy(wr_hbm, wr_ref, sem_w.at[3])
    w_cp = [pltpu.make_async_copy(src, dst, sem_w.at[4 + i]) for i, (src, dst) in enumerate(
        [(wo_hbm, wo_ref), (wg_hbm, wg_ref), (wu_hbm, wu_ref), (wd_hbm, wd_ref)])]
    o_cp = [pltpu.make_async_copy(out_scr.at[pl.ds(r0, n)], o_hbm.at[pl.ds(r0, n)], sem_o.at[c])
            for c, (r0, n) in enumerate(OUT_CHUNKS)]

    def ln_chunk(c, dep=None):
        rows = pl.ds(c * XC, XC)
        xf = x_ref[rows, :].astype(f32)
        if dep is not None:
            z = jnp.concatenate([zero_dep(pltpu.bitcast(dep, i32))] * (D // 128), axis=1)
            xf = pltpu.bitcast(pltpu.bitcast(xf, i32).reshape(XC // 8, 8, D) ^ z[None], f32).reshape(XC, D)
        mean = jnp.sum(xf, axis=-1, keepdims=True) * (1.0 / D)
        cc = xf - mean
        var = jnp.sum(cc * cc, axis=-1, keepdims=True) * (1.0 / D)
        den = rb(jnp.sqrt(rb(rb(var) + EPS_B)))
        xn = rb(rb(xf - rb(mean)) / den)
        xn_scr[rows, :] = xn.astype(bf16)
        rc = rb(jnp.sum(xn * wr_ref[...].astype(f32).reshape(1, D), axis=-1, keepdims=True))
        rowc = lax.broadcasted_iota(i32, (XC, 1), 0) + c * XC
        if c == 0:
            r_scr[...] = rc
            i_scr[...] = rowc
        else:
            rrun = r_scr[...]
            better = rc > rrun
            r_scr[...] = jnp.where(better, rc, rrun)
            i_scr[...] = jnp.where(better, rowc, i_scr[...])

    def q_chunk(c):
        rows = pl.ds(c * XC, XC)
        q = jnp.dot(xn_scr[rows, :], wqkv_ref[:, 0:D], preferred_element_type=f32)
        q_scr[:, rows] = (q * (DH ** -0.5)).T.astype(bf16)

    def kv_chunk(c):
        rows = pl.ds(c * XC, XC)
        xnb = xn_scr[rows, :]
        k = jnp.dot(xnb, wqkv_ref[:, D:2 * D], preferred_element_type=f32).astype(bf16)
        for h in range(H):
            k_scr[h, pl.ds(c * (XC // 2), XC // 2), :] = pltpu.bitcast(k[:, h * DH:(h + 1) * DH], i32)
        v = jnp.dot(xnb, wqkv_ref[:, 2 * D:3 * D], preferred_element_type=f32)
        vT_scr[:, rows] = v.T.astype(bf16)
        return v[0:8, 0:128]

    x_cp[0].start()
    wr_cp.start()
    wqkv_cp[0].start()
    x_cp[0].wait()
    wr_cp.wait()
    x_cp[1].start()
    wqkv_cp[1].start()
    wqkv_cp[2].start()
    ln_chunk(0)
    wqkv_cp[0].wait()
    x_cp[1].wait()
    ln_chunk(1)
    q_chunk(0)
    wqkv_cp[1].wait()
    wqkv_cp[2].wait()
    for c in range(2, NX):
        x_cp[c].start()
    kv_chunk(0)
    q_chunk(1)
    for c in range(2, NX):
        x_cp[c].wait()
    for cp in w_cp:
        cp.start()
    ln_chunk(2)
    vdep = kv_chunk(1)
    for c in range(2, NX):
        if c + 1 < NX:
            ln_chunk(c + 1, vdep)
        q_chunk(c)
        vdep = kv_chunk(c)

    r = r_scr[...]
    rmax = jnp.max(r, axis=0, keepdims=True)
    idx = jnp.minimum(jnp.min(jnp.where(r == rmax, i_scr[...], S)), S - 1)
    base = pl.multiple_of((idx // 16) * 16, 16)
    blk = xn_scr[pl.ds(base, 16), :]
    sel16 = lax.broadcasted_iota(i32, (16, 1), 0) == (idx - base)
    xs = jnp.where(sel16, blk, jnp.zeros_like(blk))
    moe = {'h': [], 'y': None}

    def moe_step(k):
        if k < NFP:
            cols = slice(k * FP, (k + 1) * FP)
            gg = rb(jnp.dot(xs, wg_ref[:, cols], preferred_element_type=f32))
            gg = rb(gg * jax.nn.sigmoid(gg))
            uu = rb(jnp.dot(xs, wu_ref[:, cols], preferred_element_type=f32))
            moe['h'].append((gg * uu).astype(bf16))
        else:
            j = k - NFP
            yj = jnp.dot(moe['h'][j], wd_ref[j * FP:(j + 1) * FP, :], preferred_element_type=f32)
            moe['y'] = yj if moe['y'] is None else moe['y'] + yj
            if k == 2 * NFP - 1:
                moe['y'] = rb(rb(jnp.sum(moe['y'], axis=0, keepdims=True)) * rb(jax.nn.sigmoid(rmax)))

    def out_chunk(c):
        r0, n = OUT_CHUNKS[c]
        rows = pl.ds(r0, n)
        o = oT_scr[:, rows].T.astype(bf16)
        a = jnp.dot(o, wo_ref[...], preferred_element_type=f32)
        rowc = lax.broadcasted_iota(i32, (n, 1), 0) + r0
        upd = jnp.where(rowc == idx, moe['y'], 0.0)
        out_scr[rows, :] = (x_ref[rows, :].astype(f32) + a + (xn_scr[rows, :].astype(f32) + upd)).astype(bf16)
        o_cp[c].start()

    def qk_setup(t):
        h = t // NQ
        qi = t % NQ
        if isinstance(t, int):
            return h, q_scr[h * DH:(h + 1) * DH, qi * TQ:(qi + 1) * TQ]
        qoff = pl.multiple_of(qi * TQ, TQ)
        return h, q_scr[pl.ds(pl.multiple_of(h * DH, DH), DH), pl.ds(qoff, TQ)]

    def qk_chunk(setup, buf, ci, mpart):
        h, qt = setup
        cs = ci * CK
        kh = pltpu.bitcast(k_scr[h, cs // 2:(cs + CK) // 2, :], bf16)
        s = jnp.dot(kh, qt, preferred_element_type=f32)
        buf[cs:cs + CK, :] = s
        for j in range(CK // 8):
            sj = s[j * 8:(j + 1) * 8, :]
            mpart = sj if mpart is None else jnp.maximum(mpart, sj)
        return mpart

    def fin_max(mpart):
        return jnp.broadcast_to(jnp.max(mpart, axis=0, keepdims=True), (8, TQ))

    st0 = qk_setup(0)
    st1 = qk_setup(1)
    m0 = None
    m1 = None
    for ci in range(NC + LAG):
        if ci < NC:
            m0 = qk_chunk(st0, sA, ci, m0)
        else:
            m1 = qk_chunk(st1, sB, ci - NC, m1)

    def run(t, carry, last):
        m8n, mO = carry
        nt = NL if last else NTI
        nqk = nt - 1 if last else nt + 1
        setups = [qk_setup(t + 1 + j) for j in range(nqk)]
        bufs = [sB if j % 2 == 0 else sA for j in range(nqk)]
        mp = [mO] + [None] * nt
        hist = []
        lpart = None
        ndone = 0
        for pos in range(nt * NC):
            g = pos + LAG
            ti, ci = g // NC, g % NC
            if last and pos < 2 * NFP:
                moe_step(pos)
            if ti < nqk:
                mp[ti] = qk_chunk(setups[ti], bufs[ti], ci, mp[ti])
                hist.append(mp[ti])
            else:
                hist.append(None)
                k = g - nqk * NC
                avail = ((pos // NC) + (NQ - nt)) * (TQ // XC)
                if k % 3 == 0 and ndone < avail and pos >= 2 * NFP:
                    out_chunk(ndone)
                    ndone += 1
            si, ci = pos // NC, pos % NC
            if ci == 0:
                ts = t + si
                h2 = ts // NQ
                if last:
                    hsl = slice(h2 * DH, (h2 + 1) * DH)
                    qsl = slice((ts % NQ) * TQ, (ts % NQ + 1) * TQ)
                else:
                    hsl = pl.ds(pl.multiple_of(h2 * DH, DH), DH)
                    qsl = pl.ds(pl.multiple_of((ts % NQ) * TQ, TQ), TQ)
                m8 = m8n
                lprev = lpart
                lpart = None
                acc = None
                cur = sA if si % 2 == 0 else sB
            cs = ci * CK
            w = None
            if pos - DEP >= 0 and hist[pos - DEP] is not None:
                hd = hist[pos - DEP]
                if ci - DEP == NC - 1 - LAG:
                    m8n = fin_max(hd)
                    hd = m8n
                w = pltpu.bitcast(hd, i32)
            lp = lpart if lpart is not None else lprev
            if lp is not None:
                lb = pltpu.bitcast(lp, i32)
                w = lb if w is None else w | lb
            if last and pos == 2 * NFP + 1:
                w = w | pltpu.bitcast(jnp.broadcast_to(moe['y'], (8, TQ)), i32)
            mc8 = m8
            if w is not None:
                mc8 = pltpu.bitcast(pltpu.bitcast(m8, i32) ^ zero_dep(w), f32)
            sc = cur[cs:cs + CK, :].reshape(CK // 8, 8, TQ)
            if ci == 1:
                mc8b = pltpu.bitcast(pltpu.bitcast(mc8, i32) ^ zero_dep(pltpu.bitcast(acc[0:8], i32)), f32)
                p3 = jnp.concatenate([jnp.exp(sc[:HN] - mc8b[None]), jnp.exp(sc[HN:] - mc8[None])], axis=0)
            else:
                p3 = jnp.exp(sc - mc8[None])
            for j in reversed(range(CK // 8)):
                lpart = p3[j] if lpart is None else lpart + p3[j]
            p = p3.reshape(CK, TQ)
            o = jnp.dot(vT_scr[hsl, cs:cs + CK], p.astype(bf16), preferred_element_type=f32)
            acc = o if acc is None else acc + o
            if ci == NC - 1:
                l = jnp.sum(lpart, axis=0, keepdims=True)
                oT_scr[hsl, qsl] = acc / l
        if last:
            return ndone
        return m8n, mp[nt]

    carry = lax.fori_loop(0, (NT_ - NL) // NTI, lambda i, c: run(NTI * i, c, False), (fin_max(m0), m1))
    for cp in w_cp:
        cp.wait()
    ndone = run(NT_ - NL, carry, True)
    for c in range(ndone, len(OUT_CHUNKS)):
        out_chunk(c)
    for cp in o_cp:
        cp.wait()


@jax.jit
def pallas_parallel_sum__softmax_full_mha__moe_arch_mod__prompt_kernel(
    A_x: jax.Array,
    A_wqkv: jax.Array,
    A_wo: jax.Array,
    B_x: jax.Array,
    B_w_r: jax.Array,
    B_w_gate: jax.Array,
    B_w_up: jax.Array,
    B_w_down: jax.Array,
):
    del B_x
    bf16 = jnp.bfloat16
    out = pl.pallas_call(
        _kernel,
        out_shape=jax.ShapeDtypeStruct((S, D), bf16),
        in_specs=[pl.BlockSpec(memory_space=pl.ANY)] * 7,
        out_specs=pl.BlockSpec(memory_space=pl.ANY),
        scratch_shapes=[
            pltpu.VMEM((S, D), bf16),
            pltpu.VMEM((D, 3 * D), bf16),
            pltpu.VMEM((D, D), bf16),
            pltpu.VMEM((D,), bf16),
            pltpu.VMEM((D, F), bf16),
            pltpu.VMEM((D, F), bf16),
            pltpu.VMEM((F, D), bf16),
            pltpu.VMEM((S, D), bf16),
            pltpu.VMEM((S, D), bf16),
            pltpu.VMEM((D, S), bf16),
            pltpu.VMEM((H, S // 2, DH), jnp.int32),
            pltpu.VMEM((D, S), bf16),
            pltpu.VMEM((D, S), jnp.float32),
            pltpu.VMEM((S, TQ), jnp.float32),
            pltpu.VMEM((S, TQ), jnp.float32),
            pltpu.VMEM((XC, 1), jnp.float32),
            pltpu.VMEM((XC, 1), jnp.int32),
            pltpu.SemaphoreType.DMA((NX,)),
            pltpu.SemaphoreType.DMA((8,)),
            pltpu.SemaphoreType.DMA((len(OUT_CHUNKS),)),
        ],
        compiler_params=pltpu.CompilerParams(vmem_limit_bytes=100 * 1024 * 1024),
    )(A_x.reshape(S, D), A_wqkv, A_wo, B_w_r, B_w_gate, B_w_up, B_w_down)
    return out.reshape(1, S, D)
```
